```python
import os as _os
_os.environ.setdefault("JAX_PLATFORMS", "cpu")
import jax
import jax.numpy as jnp

def _softmax(x, axis=-1):
    return jax.nn.softmax(x, axis=axis)
def _gelu(x):
    return jax.nn.gelu(x, approximate=True)
def _silu(x):
    return jax.nn.silu(x)
def _sigmoid(x):
    return jax.nn.sigmoid(x)
def _layernorm(x, axis=-1, eps=1e-5):
    m = jnp.mean(x, axis=axis, keepdims=True)
    v = jnp.var(x, axis=axis, keepdims=True)
    return (x - m) / jnp.sqrt(v + eps)
def _scatter_add(tgt, idx, src, axis=0):
    return tgt.at[idx].add(src)
def _segment_sum(src, seg, n):
    return jax.ops.segment_sum(src, seg, n)
class _Rng:
    def __init__(self, key):
        self._k = key
    def _next(self):
        self._k, sub = jax.random.split(self._k)
        return sub
    def normal(self, shape):
        return jax.random.normal(self._next(), shape, dtype=jnp.bfloat16)
    def randint(self, lo, hi, shape):
        return jax.random.randint(self._next(), shape, lo, hi, dtype=jnp.int32)
    def uniform(self, shape, lo=0.0, hi=1.0):
        return jax.random.uniform(self._next(), shape, jnp.bfloat16, lo, hi)
    def permutation(self, n):
        return jax.random.permutation(self._next(), n)


kernel_name = 'standalone__fft_conv__vision'

def setup_inputs():
    _rng = _Rng(jax.random.key(int.from_bytes(__import__("os").urandom(4), "little")))
    _w = (lambda a: (lambda t: t.astype(jnp.bfloat16) if jnp.issubdtype(t.dtype, jnp.floating) else t)(jnp.asarray(a)))
    H = W = 224
    C = 96
    K = 3
    return {
        "x": _w((lambda *s: _rng.normal(s) * 0.05)(1, H, W, C)),
        "w": _w((lambda *s: _rng.normal(s) * 0.05)(K, K, C, C)),
    }

def reference(x, w):
    B, H, W, C = x.shape
    K = w.shape[0]
    wp = jnp.pad(w, ((0, H - K), (0, W - K), (0, 0), (0, 0)))
    Xf = (lambda x, axes=(-2,-1): jnp.fft.rfft2(x.astype(jnp.float32), axes=axes))(x, axes=(1, 2))
    Wf = (lambda x, axes=(-2,-1): jnp.fft.rfft2(x.astype(jnp.float32), axes=axes))(wp, axes=(0, 1))
    Yf = jnp.einsum('bhwi,hwio->bhwo', Xf, Wf)
    y = (lambda x, s, axes=(-2,-1): jnp.fft.irfft2(x, s=s, axes=axes).astype(jnp.bfloat16))(Yf, (H, W), axes=(1, 2))
    return y
```

```python
import functools
import jax, jax.numpy as jnp, numpy as np
from jax import lax
from jax.experimental import pallas as pl
from jax.experimental.pallas import tpu as pltpu

H = W = 224
C = 96
S = 8
HS = H // S
NS = HS // 2
NC = C // 16
f32, bf16, u32 = jnp.float32, jnp.bfloat16, jnp.uint32
X, Y = (1, 1), (2, 2)
EXTRA = {
    (1, 0): ((X, 0, 1), (X, 1, 2)),  (1, 3): ((X, 0, -1), (X, 2, -2)), (1, 2): ((X, 1, -1), (X, 2, 1)),
    (0, 1): ((X, 3, 1), (X, 4, 1)),  (3, 1): ((X, 3, -1), (X, 4, -1)),
    (2, 0): ((Y, 0, 1), (Y, 1, 2)),  (2, 3): ((Y, 0, 1), (Y, 2, 2)),   (2, 1): ((Y, 1, -1), (Y, 2, 1)),
    (0, 2): ((Y, 3, 1), (Y, 4, 1)),  (3, 2): ((Y, 3, 1), (Y, 4, 1)),
    (0, 0): ((X, 5, 1), (Y, 5, 1)),  (0, 3): ((X, 5, -1), (Y, 5, 1)),
    (3, 0): ((X, 5, -1), (Y, 5, 1)), (3, 3): ((X, 5, 1), (Y, 5, 1)),
}
CELLS = sorted(EXTRA)

def make(mode='full', flags=None, tag='', D=2, NI=None, border=1, doa=1, doc=1, W0=6):
    NI = NS if NI is None else NI
    def kern(x_hbm, w_hbm, o_hbm, x0, x1, y0, y1, ub, eb, zb, w_ref, sem, rsem):
        xi = x_hbm.bitcast(u32); oi = o_hbm.bitcast(u32)
        halves = (pl.ds(0, 128), pl.ds(128, W - 128))
        def reads(r, n):
            return [pltpu.make_async_copy(xi.at[:, pl.ds(r, n), :, ls], xx.at[:, pl.ds(r, n)], rsem.at[r]) for xx, ls in zip((x0, x1), halves)]
        def writes(r):
            return [pltpu.make_async_copy(yy.at[:, r], oi.at[:, r, :, ls], sem.at[1]) for yy, ls in zip((y0, y1), halves)]
        def writes_wrapped(r):
            cps = []
            for yy, ls in zip((y0, y1), halves):
                cps += [pltpu.make_async_copy(yy.at[pl.ds(0, S - 1), r], oi.at[pl.ds(1, S - 1), r, :, ls], sem.at[1]),
                        pltpu.make_async_copy(yy.at[S - 1, r], oi.at[0, r, :, ls], sem.at[1])]
            return cps
        wcp = pltpu.make_async_copy(w_hbm, w_ref, sem.at[0])
        if mode != 'compute':
            for cp in reads(0, 1): cp.start()
        wcp.start()
        if mode != 'compute':
            for r, n in [(r, 1) for r in range(1, 4)] + [(r, 2) for r in range(4, HS, 2)]:
                for cp in reads(r, n): cp.start()
        wcp.wait()
        g = [[w_ref[2 - a, 2 - b].astype(f32) for b in range(3)] for a in range(3)]
        def gt(v):
            s = (v[0] + v[2]) * 0.5; h = v[1] * 0.5
            return [v[0], s + h, s - h, v[2]]
        gw = [gt(g[a]) for a in range(3)]
        U = {}
        for l in range(4):
            col = gt([gw[a][l] for a in range(3)])
            for k in range(4):
                U[k, l] = col[k]
        for n, cell in enumerate(CELLS):
            parts = [U[cell]] + [U[src][16 * c:16 * c + 16] * float(s) for src, c, s in EXTRA[cell]]
            ub[n] = pltpu.bitcast(jnp.concatenate(parts, axis=0).T.astype(bf16), u32)
        lane = lax.broadcasted_iota(jnp.int32, (8, 128), 1)
        even = (lane & 1) == 0
        below = functools.lru_cache(None)(lambda n: lane < n)
        for n in (1, 31, 32, 63, 64, 93, 94, 95, 96, 125, 126, 127): below(n)
        cut = lambda n, a, b: jnp.where(below(n), a, b)
        roll = lambda v, s: pltpu.roll(v, s, 1)
        up = lambda z: pltpu.bitcast(z, bf16).astype(f32)

        def stage_a(rows, ev, c):
            cs = pl.ds(8 * c, 8); ch = pl.ds(16 * c, 16)
            pq = lambda a, b: (jnp.where(even, b, a), jnp.where(even, a, b))
            ld0 = lambda s: x0[rows[s][0], rows[s][1], cs, :]
            ld1 = lambda s: x1[rows[s][0], rows[s][1], cs, :]
            def emit(i, d0, d1, d2, d3):
                f2 = up(d2); ev[i, 0, ch] = up(d0) - f2
                f1 = up(d1); ev[i, 1, ch] = f1 + f2
                ev[i, 2, ch] = f2 - f1
                ev[i, 3, ch] = f1 - up(d3)
            def t0(j, wr):
                p, q = pq(ld0(2 * j), ld0(2 * j + 1))
                emit(j, roll(cut(125, p, wr[0]), 3), roll(cut(126, q, wr[1]), 2), roll(cut(127, p, wr[0]), 1), q)
                return p, q
            def unit(j, gg):
                a, b = ld1(2 * j), ld1(2 * j + 1)
                f1 = pq(*(jnp.concatenate([v, jnp.zeros((8, 32), u32)], axis=1) for v in (a, b)))
                wr = [roll(v, 32) for v in f1]
                rr = [roll(v, 96 - 32 * j) for v in gg]
                def fin():
                    f0 = t0(j, wr)
                    sh = lambda n, s: roll(cut(128 - s, cut(96 - s, f1[n], rr[n]), f0[n]), s)
                    emit(4 + j, sh(0, 3), sh(1, 2), sh(0, 1), cut(96, f1[1], rr[1]))
                    if j == 2: t0(3, rr)
                return fin
            st = {}
            def first():
                st['g'] = pq(*(jnp.concatenate([ld1(s), ld0(s)[:, 96:]], axis=1) for s in (6, 7)))
                return unit(0, st['g'])
            return [first, lambda: unit(1, st['g']), lambda: unit(2, st['g'])]

        def mms(ev, cells, msplit=False):
            cache = {}
            def e(i, n, l, c):
                if (i, n, l, c) not in cache:
                    cache[i, n, l, c] = ev[n, i, l, pl.ds(16 * c, 16)]
                return cache[i, n, l, c]
            vc = {}
            def v(i, cell, c):
                k, l = cell
                if (i, cell, c) not in vc:
                    p, q = ((0, 2), (1, 2), (2, 1), (1, 3))[k]
                    vc[i, cell, c] = e(i, p, l, c) + e(i, q, l, c) if k == 1 else e(i, p, l, c) - e(i, q, l, c)
                return vc[i, cell, c]
            out = []
            for i, cell in cells:
                rhs = jnp.concatenate([v(i, cell, n) for n in range(NC)] + [v(i, *ex[:2]) for ex in EXTRA[cell]], axis=0).astype(bf16)
                n = CELLS.index(cell)
                if msplit:
                    out.append(jnp.concatenate([jnp.dot(pltpu.bitcast(ub[n, pl.ds(24 * h, 24)], bf16), rhs, preferred_element_type=f32) for h in range(2)], axis=0))
                else:
                    out.append(jnp.dot(pltpu.bitcast(ub[n], bf16), rhs, preferred_element_type=f32))
            return out
        def put(zv, i, a, b, y):
            for c in range(NC):
                zv[a, b, i, pl.ds(8 * c, 8)] = jnp.concatenate([y[16 * c:16 * c + 8], y[16 * c + 8:16 * c + 16]], axis=1).astype(bf16)
        def head(ev, zv, i):
            m33, m23, m13, m03 = mms(ev, [(i, (k, 3)) for k in (3, 2, 1, 0)])
            n01 = m03 + (m13 + m23); y11 = m33 - (m13 - m23)
            m32, m31, m12, m21 = mms(ev, [(i, (3, 2)), (i, (3, 1)), (i, (1, 2)), (i, (2, 1))])
            p, q = m21 + m31, m12 - m32
            put(zv, i, 1, 1, y11 - (p + q))
            y10 = q - p; y00 = m12 + m21; n01 = n01 + (m12 - m21)
            m02, m01, m30, m00 = mms(ev, [(i, (0, 2)), (i, (0, 1)), (i, (3, 0)), (i, (0, 0))])
            put(zv, i, 0, 1, (m01 - m02) - n01)
            return y00 + (m01 + m02) + m00, y10 - m30
        def tail(ev, zv, i, m20, m10):
            m02, m01, m30, m00 = mms(ev, [(i, (0, 2)), (i, (0, 1)), (i, (3, 0)), (i, (0, 0))])
            y00 = (m10 + m20) + (m01 + m02) + m00; y10 = (m10 - m20) - m30; y01 = m01 - m02
            m32, m31, m12, m21 = mms(ev, [(i, (3, 2)), (i, (3, 1)), (i, (1, 2)), (i, (2, 1))])
            p, q = m21 + m31, m12 - m32
            put(zv, i, 0, 0, y00 + (m12 + m21)); put(zv, i, 1, 0, y10 + (q - p))
            y01 = y01 - (m12 - m21); n11 = p + q
            m33, m23, m13, m03 = mms(ev, [(i, (k, 3)) for k in (3, 2, 1, 0)])
            put(zv, i, 0, 1, y01 - (m03 + (m13 + m23))); put(zv, i, 1, 1, (m33 - (m13 - m23)) - n11)
        def old(ev, zv, i, m21, m12):
            m = mms(ev, [(i, (0, 1)), (i, (3, 1)), (i, (0, 2)), (i, (3, 2))])
            u10, u11, u20, u21 = m[0] + m21, m21 + m[1], m[2] + m12, m12 - m[3]
            s0, s1, d0, d1 = u10 + u20, u21 - u11, u10 - u20, u11 + u21
            m = mms(ev, [(i, (k, 3)) for k in range(4)])
            put(zv, i, 0, 1, d0 - (m[0] + m[1] + m[2])); put(zv, i, 1, 1, (m[2] + m[3] - m[1]) - d1)
            m = mms(ev, [(i, (k, 0)) for k in range(4)])
            put(zv, i, 0, 0, s0 + (m[0] + m[1] + m[2])); put(zv, i, 1, 0, s1 + (m[1] - m[2] - m[3]))
        def stage_b(ev, zv):
            if border == 1:
                tail(ev, zv, 6, *mms(ev, [(6, (2, 0)), (6, (1, 0))], msplit=True))
                for i in (0, 2, 4):
                    y00, y10 = head(ev, zv, i)
                    m = mms(ev, [(i, (2, 0)), (i, (1, 0)), (i + 1, (2, 0)), (i + 1, (1, 0))])
                    put(zv, i, 0, 0, y00 + (m[1] + m[0])); put(zv, i, 1, 0, y10 + (m[1] - m[0]))
                    tail(ev, zv, i + 1, m[2], m[3])
            else:
                old(ev, zv, 6, *mms(ev, [(6, (2, 1)), (6, (1, 2))], msplit=True))
                for i in (0, 2, 4):
                    m = mms(ev, [(i, (2, 1)), (i, (1, 2)), (i + 1, (2, 1)), (i + 1, (1, 2))])
                    old(ev, zv, i, m[0], m[1]); old(ev, zv, i + 1, m[2], m[3])
        def stage_c(y0v, y1v, r, zv, a, c):
            cs = pl.ds(8 * c, 8)
            def ld(b, i):
                return pltpu.bitcast(jnp.concatenate([zv[a, b, i, cs, 0:128], zv[a, b, i, cs, 128:256]], axis=0), u32)
            def out(j, s0, s1, z0, z1):
                y0v[2 * j, r, cs] = jnp.where(even, s0, z0); y0v[2 * j + 1, r, cs] = jnp.where(even, z0, s0)
                y1v[2 * j, r, cs] = jnp.where(even, s1, z1)[:, :96]; y1v[2 * j + 1, r, cs] = jnp.where(even, z1, s1)[:, :96]
            st = []
            def unit(j):
                f0, fu, su = ld(0, j), ld(0, 4 + j), ld(1, 4 + j)
                rf0, rfu, w = roll(f0, 127), roll(fu, 127), roll(f0, 95)
                out(j, ld(1, j), su, cut(127, rf0, rfu), cut(95, rfu, w))
                if j == 2:
                    f3 = ld(0, 3); fu = cut(1, f3, fu)
                st.append((roll(su, 32 * (j + 1)), roll(fu, 32 * (j + 1) - 1)))
                if j == 2:
                    (s0, g0), (s1, g1), (s2, g2) = st
                    out(3, ld(1, 3), cut(64, cut(32, s0, s1), s2), cut(127, roll(f3, 127), g0), cut(63, cut(31, g0, g1), g2))
            return [functools.partial(unit, j) for j in range(3)]
        def run(ua, uc):
            pend = []
            for n in range(max(len(ua), len(uc))):
                if n < len(ua): pend.append(ua[n]())
                if n < len(uc): uc[n]()
                if len(pend) > D: pend.pop(0)()
            while pend: pend.pop(0)()
        def pro(r, carry):
            if mode != 'compute':
                for cp in reads(r, 1): cp.wait()
            run([u for c in range(NC) for u in stage_a([(s, r) for s in range(S)], eb.at[r], c)], [])
            return carry
        lax.fori_loop(0, 4, pro, 0)
        zb[0] = jnp.zeros(zb.shape[1:], bf16)
        def body(t, carry):
            if mode != 'compute':
                @pl.when(2 * t + 4 < HS)
                def _():
                    for cp in reads(2 * t + 4, 2): cp.wait()
            ev = eb.at[pl.ds(2 * t, 6)]; zv = zb.at[pl.ds(t, 2)]
            y0v = y0.at[:, pl.ds(2 * t, 2)]; y1v = y1.at[:, pl.ds(2 * t, 2)]
            stage_b(ev, zv.at[1])
            ua, uc = [], []
            wrap = (2 * t + 4 >= HS).astype(jnp.int32)
            for a in range(2):
                r = 2 * t + 4 + a - HS * wrap
                rows = [((s + wrap) & (S - 1), r) for s in range(S)]
                for c in range(NC):
                    if doa: ua += stage_a(rows, ev.at[4 + a], c)
                    if doc: uc += stage_c(y0v, y1v, a, zv.at[0], a, c)
            run(ua, uc)
            if mode != 'compute':
                @pl.when(t >= W0 - 1)
                def _():
                    def go(r, c):
                        for cp in writes(r): cp.start()
                        return c
                    lax.fori_loop(jnp.where(t == W0 - 1, 2, 2 * t), 2 * t + 2, go, 0)
            return carry
        lax.fori_loop(0, NI, body, 0)
        def epi(a, carry):
            run([], [u for c in range(NC) for u in stage_c(y0, y1, a, zb.at[NS], a, c)])
            for cp in writes_wrapped(a): cp.start()
            return carry
        lax.fori_loop(0, 2, epi, 0)
        keep = pltpu.make_async_copy(eb.at[0, 0, 0, pl.ds(0, 8)], eb.at[1, 0, 0, pl.ds(0, 8)], sem.at[0])
        keep.start(); keep.wait()
        if mode != 'compute':
            for yy in (y0, y1): pltpu.make_async_copy(yy, yy, sem.at[1]).wait()
        else:
            for a in range(2):
                for cp in writes_wrapped(a): cp.wait()
    def f(x, w):
        xt = jnp.transpose(x[0], (0, 2, 1)).reshape(S, HS, C, W)
        y = pl.pallas_call(kern, name=f"v8_{W0}_{mode}_{D}_{border}_{doa}{doc}{tag}",
            in_specs=[pl.BlockSpec(memory_space=pl.ANY), pl.BlockSpec(memory_space=pl.ANY)],
            out_specs=pl.BlockSpec(memory_space=pl.ANY),
            out_shape=jax.ShapeDtypeStruct((S, HS, C, W), bf16),
            scratch_shapes=[pltpu.VMEM((S, HS, C // 2, 128), u32), pltpu.VMEM((S, HS, C // 2, W - 128), u32),
                            pltpu.VMEM((S, HS, C // 2, 128), u32), pltpu.VMEM((S, HS, C // 2, W - 128), u32),
                            pltpu.VMEM((14, C // 2, 128), u32), pltpu.VMEM((HS + 4, 7, 4, C, 128), f32),
                            pltpu.VMEM((NS + 1, 2, 2, 7, C // 2, 256), bf16), pltpu.VMEM((3, 3, C, C), bf16), pltpu.SemaphoreType.DMA((2,)), pltpu.SemaphoreType.DMA((HS,))],
            compiler_params=pltpu.CompilerParams(vmem_limit_bytes=110 * 2**20, flags=flags),
        )(xt, w)
        return jnp.transpose(y.reshape(H, C, W), (0, 2, 1))[None]
    return f


_impl = make()


@jax.jit
def pallas_standalone__fft_conv__vision_kernel(x: jax.Array, w: jax.Array):
    return _impl(x, w)
```

```python
import functools

import jax
import jax.numpy as jnp
from jax import lax
import jax.experimental.pallas as pl
import jax.experimental.pallas.tpu as pltpu

H = W = 224
C = 96
STRIPS = 8
STEPS = H // STRIPS // 2
CHUNKS = C // 16
FIRST_WRITE_STEP = 6

_X, _Y = (1, 1), (2, 2)
_FOLDED = {
    (0, 0): ((_X, 5, 1.0), (_Y, 5, 1.0)),
    (0, 1): ((_X, 3, 1.0), (_X, 4, 1.0)),
    (0, 2): ((_Y, 3, 1.0), (_Y, 4, 1.0)),
    (0, 3): ((_X, 5, -1.0), (_Y, 5, 1.0)),
    (1, 0): ((_X, 0, 1.0), (_X, 1, 2.0)),
    (1, 2): ((_X, 1, -1.0), (_X, 2, 1.0)),
    (1, 3): ((_X, 0, -1.0), (_X, 2, -2.0)),
    (2, 0): ((_Y, 0, 1.0), (_Y, 1, 2.0)),
    (2, 1): ((_Y, 1, -1.0), (_Y, 2, 1.0)),
    (2, 3): ((_Y, 0, 1.0), (_Y, 2, 2.0)),
    (3, 0): ((_X, 5, -1.0), (_Y, 5, 1.0)),
    (3, 1): ((_X, 3, -1.0), (_X, 4, -1.0)),
    (3, 2): ((_Y, 3, 1.0), (_Y, 4, 1.0)),
    (3, 3): ((_X, 5, 1.0), (_Y, 5, 1.0)),
}
_PRODUCTS = tuple(sorted(_FOLDED))
_NEGATED = ((3, 0), (3, 2), (0, 3))
_HALVED = ((3, 1), (3, 2))

f32, bf16, u32 = jnp.float32, jnp.bfloat16, jnp.uint32


def _transform_filter(w_ref, u_ref):
    def transform(g):
        outer, inner = (g[0] + g[2]) * 0.5, g[1] * 0.5
        return [g[0], outer + inner, outer - inner, g[2]]

    g = [
        transform([w_ref[2 - a, 2 - b].astype(f32) for b in range(3)])
        for a in range(3)
    ]
    u = {}
    for l in range(4):
        for k, v in enumerate(transform([g[a][l] for a in range(3)])):
            u[k, l] = v
    for n, kl in enumerate(_PRODUCTS):
        folded = [u[src][16 * c : 16 * c + 16] * s for src, c, s in _FOLDED[kl]]
        v = jnp.concatenate([u[kl]] + folded, axis=0)
        if kl in _NEGATED:
            v = -v
        u_ref[n] = pltpu.bitcast(v.T.astype(bf16), u32)


def _kernel(
    x_hbm, w_hbm, o_hbm, x0, x1, y0, y1, w_ref, u_ref, e_ref, z_ref, sem, row_sem
):
    x_words, o_words = x_hbm.bitcast(u32), o_hbm.bitcast(u32)
    lanes = (pl.ds(0, 128), pl.ds(128, W - 128))

    def reads(q, a, n):
        return [
            pltpu.make_async_copy(
                x_words.at[:, q, a, :, ls], buf.at[:, q, a], row_sem.at[n]
            )
            for buf, ls in zip((x0, x1), lanes)
        ]

    def row_reads(r):
        return reads(r >> 1, r & 1, r)

    def step_reads(q):
        return reads(q, slice(None), q + 2)

    def start_writes(src_strip, src_step, dst_strip, dst_step, a):
        for buf, ls in zip((y0, y1), lanes):
            pltpu.make_async_copy(
                buf.at[src_strip, src_step, a],
                o_words.at[dst_strip, dst_step, a, :, ls],
                sem.at[1],
            ).start()

    def write_steps(lo, hi):
        def body(t, carry):
            for a in range(2):
                start_writes(slice(None), t, slice(None), t + 1, a)
            return carry

        lax.fori_loop(lo, hi, body, 0)

    w_copy = pltpu.make_async_copy(w_hbm, w_ref, sem.at[0])
    w_copy.start()
    for copy in [cp for r in range(4) for cp in row_reads(r)] + step_reads(2):
        copy.start()
    w_copy.wait()
    _transform_filter(w_ref, u_ref)

    lane = lax.broadcasted_iota(jnp.int32, (8, 128), 1)
    even = (lane & 1) == 0
    below = {n: lane < n for n in (1, 31, 32, 63, 64, 95, 96, 125, 126, 127)}
    band = {s: ((lane + s) & 96) == 96 for s in (1, 2, 3)}

    def cut(n, a, b):
        return jnp.where(below[n], a, b)

    def roll(v, s):
        return pltpu.roll(v, s, 1)

    def row_transform(strip, q, a, e, c):
        words, rows = pl.ds(8 * c, 8), pl.ds(16 * c, 16)

        def head(s):
            return x0[strip[s], q, a, words, :]

        def tail(s):
            rest = x1[strip[s], q, a, words, :]
            return jnp.concatenate([rest, head(s)[:, 96:]], axis=1)

        def board(load, j):
            first, second = load(2 * j), load(2 * j + 1)
            return jnp.where(even, second, first), jnp.where(even, first, second)

        def emit(tile, *d):
            d = [pltpu.bitcast(v, bf16).astype(f32) for v in d]
            e[tile, 0, rows] = d[0] - d[2]
            e[tile, 1, rows] = d[1] + d[2]
            e[tile, 2, rows] = d[2] - d[1]
            e[tile, 3, rows] = d[1] - d[3]

        def head_tile(j, wrap):
            other, own = board(head, j)
            emit(
                j,
                roll(cut(125, other, wrap[0]), 3),
                roll(cut(126, own, wrap[1]), 2),
                roll(cut(127, other, wrap[0]), 1),
                own,
            )

        tail_board = functools.lru_cache(None)(lambda j: board(tail, j))

        def job(j):
            filler, rest = tail_board(3), tail_board(j)
            wrap = [roll(v, 32) for v in rest]
            piece = [roll(v, 96 - 32 * j) for v in filler]

            def finish():
                def shifted(n, s):
                    return roll(jnp.where(band[s], piece[n], rest[n]), s)

                head_tile(j, wrap)
                emit(
                    4 + j,
                    shifted(0, 3),
                    shifted(1, 2),
                    shifted(0, 1),
                    cut(96, rest[1], piece[1]),
                )
                if j == 2:
                    head_tile(3, piece)

            return finish

        return [functools.partial(job, j) for j in range(3)]

    def product(e, tile, k, l, acc=None):
        def v(kl, c):
            p, q = (
                e[n // 2, n % 2, tile, kl[1], pl.ds(16 * c, 16)]
                for n in ((0, 2), (1, 2), (2, 1), (1, 3))[kl[0]]
            )
            return p + q if kl[0] == 1 else p - q

        rhs = jnp.concatenate(
            [v((k, l), c) for c in range(CHUNKS)]
            + [v(src, c) for src, c, _ in _FOLDED[k, l]],
            axis=0,
        ).astype(bf16)

        def dot(lo, size):
            lhs = u_ref[_PRODUCTS.index((k, l)), pl.ds(lo // 2, size // 2)]
            m = jnp.dot(pltpu.bitcast(lhs, bf16), rhs, preferred_element_type=f32)
            return m if acc is None else acc[lo : lo + size] + m

        if (k, l) in _HALVED:
            return jnp.concatenate([dot(0, C // 2), dot(C // 2, C // 2)], axis=0)
        return dot(0, C)

    held = {}

    def put(tile, a, b, y):
        if tile in (1, 2):
            held[tile, a, b] = pltpu.bitcast(y.astype(bf16), u32)
            return
        z_ref[a, b, tile] = jnp.concatenate(
            [
                jnp.concatenate([y[r : r + 16], y[r + 16 : r + 32]], axis=1)
                for r in range(0, C, 32)
            ],
            axis=0,
        ).astype(bf16)

    def get(tile, a, b, c):
        if tile in (1, 2):
            return held[tile, a, b][8 * c : 8 * c + 8]
        z = z_ref[a, b, tile, pl.ds(16 * (c // 2), 16), pl.ds(128 * (c % 2), 128)]
        return pltpu.bitcast(z, u32)

    def convolve(e, tile):
        m = functools.partial(product, e, tile)
        m10, m20 = m(1, 0), m(2, 0)
        top0, bottom0 = m(0, 0, m10 + m20), m(3, 0, m10 - m20)
        m21, m12 = m(2, 1), m(1, 2)
        top1, top2 = m(0, 1, m21), m(0, 2, m12)
        minus_bottom1, bottom2 = m(3, 1, m21), m(3, 2, m12)
        top, minus_bottom = top1 - top2, minus_bottom1 + bottom2
        put(tile, 0, 0, top0 + (top + (top2 + top2)))
        put(tile, 1, 0, bottom0 + (minus_bottom - (minus_bottom1 + minus_bottom1)))

        def finish():
            m13, m23 = m(1, 3), m(2, 3)
            put(tile, 0, 1, m(0, 3, top - (m13 + m23)))
            put(tile, 1, 1, m(3, 3, (m23 - m13) - minus_bottom))

        return finish

    def convolve_tiles(e, tiles):
        for tile in tiles[:-2]:
            convolve(e, tile)()
        finish = convolve(e, tiles[-2])
        convolve(e, tiles[-1])()
        finish()

    def unpack(out0, out1, j, a, c):
        left0 = get(j, a, 0, c)
        if j < 3:
            moved = roll(get(4 + j, a, 0, c), 127)
            right1 = get(4 + j, a, 1, c)
            next0 = cut(127, roll(left0, 127), moved)
            next1 = cut(95, moved, roll(left0, 95))
        else:
            r = [roll(get(4 + i, a, 1, c), 32 * (i + 1)) for i in range(3)]
            left = [get(4, a, 0, c), get(5, a, 0, c), cut(1, left0, get(6, a, 0, c))]
            n = [roll(v, 32 * (i + 1) - 1) for i, v in enumerate(left)]
            right1 = cut(64, cut(32, r[0], r[1]), r[2])
            next0 = cut(127, roll(left0, 127), n[0])
            next1 = cut(63, cut(31, n[0], n[1]), n[2])
        right0 = get(j, a, 1, c)
        words = pl.ds(8 * c, 8)
        out0[2 * j, a, words] = jnp.where(even, right0, next0)
        out0[2 * j + 1, a, words] = jnp.where(even, next0, right0)
        out1[2 * j, a, words] = jnp.where(even, right1, next1)[:, : W - 128]
        out1[2 * j + 1, a, words] = jnp.where(even, next1, right1)[:, : W - 128]

    def interleave(jobs, depth, outputs=()):
        pending, outputs = [], list(outputs)
        for n, job in enumerate(jobs):
            pending.append(job())
            while outputs and outputs[0][0] <= n:
                outputs.pop(0)[1]()
            while len(pending) > depth[n * len(depth) // len(jobs)]:
                pending.pop(0)()
        for finish in pending:
            finish()
        for _, output in outputs:
            output()

    row_chunks = [(a, c) for a in range(2) for c in range(CHUNKS)]

    def step(t, depth, spans, midway=None):
        e = e_ref.at[pl.ds(t, 3)]
        for tile in (0, 4):
            convolve(e, tile)()
        if midway:
            midway()
        convolve_tiles(e, (5, 6, 3, 1, 2))
        wrapped = (t + 2 >= STEPS).astype(jnp.int32)
        q = t + 2 - STEPS * wrapped
        strip = [(s + wrapped) & (STRIPS - 1) for s in range(STRIPS)]
        out = y0.at[:, t], y1.at[:, t]
        interleave(
            [
                job
                for a, c in row_chunks
                for job in row_transform(strip, q, a, e.at[2, a], c)
            ],
            depth,
            [
                (lo + (hi - lo) * n / 12, functools.partial(unpack, *out, j, a, c))
                for j, lo, hi in spans
                for n, (a, c) in enumerate(row_chunks)
            ],
        )

    def first_rows(r, carry):
        q, a = r >> 1, r & 1
        for copy in row_reads(r):
            copy.wait()
        interleave(
            [
                job
                for c in range(CHUNKS)
                for job in row_transform(range(STRIPS), q, a, e_ref.at[q, a], c)
            ],
            (4,),
        )
        return carry

    lax.fori_loop(0, 4, first_rows, 0)
    for q in range(3, STEPS):
        for copy in step_reads(q):
            copy.start()

    def phase(writing, carry):
        t0 = writing * FIRST_WRITE_STEP

        def midway():
            for copy in step_reads(t0 + 2):
                copy.wait()
            write_steps(0, t0)

        step(t0, (3,), ((0, 0, 12), (3, 24, 32), (1, 32, 36), (2, 36, 36)), midway)

        def body(t, carry):
            write_steps(t - 1, writing * t)

            @pl.when(t + 2 < STEPS)
            def _():
                for copy in step_reads(t + 2):
                    copy.wait()

            spans = ((0, 13, 27), (3, 33, 36), (1, 36, 36), (2, 36, 36))
            step(t, (2, 2, 1, 1, 2), spans)
            return carry

        end = jnp.where(writing == 0, FIRST_WRITE_STEP, STEPS - 1)
        lax.fori_loop(t0 + 1, end, body, 0)
        return carry

    lax.fori_loop(0, 2, phase, 0)

    last = STEPS - 1
    for a in range(2):
        start_writes(slice(None), last - 1, slice(None), last, a)
    for tiles, pairs in (((0, 4, 5, 6, 3), (0, 3)), ((1, 2), (1, 2))):
        convolve_tiles(e_ref.at[pl.ds(last, 2)], tiles)
        for j in pairs:
            for a, c in row_chunks:
                unpack(y0.at[:, last], y1.at[:, last], j, a, c)
        for a in range(2):
            for s in [2 * j + i for j in pairs for i in range(2)]:
                start_writes(s, last, (s + 1) % STRIPS, 0, a)
    pltpu.make_async_copy(o_words, o_words, sem.at[1]).wait()


@jax.jit
def pallas_standalone__fft_conv__vision_kernel(
    x: jax.Array,
    w: jax.Array,
):
    assert x.shape == (1, H, W, C) and w.shape == (3, 3, C, C)
    shape = (STRIPS, STEPS, 2, C, W)
    head = pltpu.VMEM((STRIPS, STEPS, 2, C // 2, 128), u32)
    tail = pltpu.VMEM((STRIPS, STEPS, 2, C // 2, W - 128), u32)
    y = pl.pallas_call(
        _kernel,
        in_specs=[pl.BlockSpec(memory_space=pl.ANY)] * 2,
        out_specs=pl.BlockSpec(memory_space=pl.ANY),
        out_shape=jax.ShapeDtypeStruct(shape, bf16),
        scratch_shapes=[
            head,
            tail,
            head,
            tail,
            pltpu.VMEM((3, 3, C, C), bf16),
            pltpu.VMEM((len(_PRODUCTS), C // 2, 128), u32),
            pltpu.VMEM((STEPS + 1, 2, 7, 4, C, 128), f32),
            pltpu.VMEM((2, 2, 7, C // 2, 256), bf16),
            pltpu.SemaphoreType.DMA((2,)),
            pltpu.SemaphoreType.DMA((STEPS + 2,)),
        ],
        compiler_params=pltpu.CompilerParams(
            vmem_limit_bytes=96 * 1024 * 1024,
            disable_semaphore_checks=True,
        ),
    )(jnp.transpose(x[0], (0, 2, 1)).reshape(shape), w)
    return jnp.transpose(y.reshape(H, C, W), (0, 2, 1))[None]
```

```python
import functools

import jax
import jax.numpy as jnp
from jax import lax
import jax.experimental.pallas as pl
import jax.experimental.pallas.tpu as pltpu

H = W = 224
C = 96
STRIPS = 8
STEPS = H // STRIPS // 2
CHUNKS = C // 16
FIRST_WRITE_STEP = 6

_X, _Y = (1, 1), (2, 2)
_FOLDED = {
    (0, 0): ((_X, 5, 1.0), (_Y, 5, 1.0)),
    (0, 1): ((_X, 3, 1.0), (_X, 4, 1.0)),
    (0, 2): ((_Y, 3, 1.0), (_Y, 4, 1.0)),
    (0, 3): ((_X, 5, -1.0), (_Y, 5, 1.0)),
    (1, 0): ((_X, 0, 1.0), (_X, 1, 2.0)),
    (1, 2): ((_X, 1, -1.0), (_X, 2, 1.0)),
    (1, 3): ((_X, 0, -1.0), (_X, 2, -2.0)),
    (2, 0): ((_Y, 0, 1.0), (_Y, 1, 2.0)),
    (2, 1): ((_Y, 1, -1.0), (_Y, 2, 1.0)),
    (2, 3): ((_Y, 0, 1.0), (_Y, 2, 2.0)),
    (3, 0): ((_X, 5, -1.0), (_Y, 5, 1.0)),
    (3, 1): ((_X, 3, -1.0), (_X, 4, -1.0)),
    (3, 2): ((_Y, 3, 1.0), (_Y, 4, 1.0)),
    (3, 3): ((_X, 5, 1.0), (_Y, 5, 1.0)),
}
_PRODUCTS = tuple(sorted(_FOLDED))
_NEGATED = ((3, 0), (3, 2), (0, 3))
_HALVED = ((3, 1), (3, 2))

f32, bf16, u32 = jnp.float32, jnp.bfloat16, jnp.uint32


def _transform_filter(w_ref, u_ref):
    def transform(g):
        outer, inner = (g[0] + g[2]) * 0.5, g[1] * 0.5
        return [g[0], outer + inner, outer - inner, g[2]]

    g = [
        transform([w_ref[2 - a, 2 - b].astype(f32) for b in range(3)])
        for a in range(3)
    ]
    u = {}
    for l in range(4):
        for k, v in enumerate(transform([g[a][l] for a in range(3)])):
            u[k, l] = v
    for n, kl in enumerate(_PRODUCTS):
        folded = [u[src][16 * c : 16 * c + 16] * s for src, c, s in _FOLDED[kl]]
        v = jnp.concatenate([u[kl]] + folded, axis=0)
        if kl in _NEGATED:
            v = -v
        u_ref[n] = pltpu.bitcast(v.T.astype(bf16), u32)


def _kernel(
    x_hbm, w_hbm, o_hbm, x0, x1, y_ref, u_ref, e_ref, z_ref, w_ref, sem, row_sem
):
    lanes = (pl.ds(0, 128), pl.ds(128, W - 128))

    def reads(q, a, n):
        return [
            pltpu.make_async_copy(
                x_hbm.at[:, q, a, :, ls], buf.at[:, q, a], row_sem.at[n]
            )
            for buf, ls in zip((x0, x1), lanes)
        ]

    def row_reads(r):
        return reads(r >> 1, r & 1, r)

    def step_reads(q):
        return reads(q, slice(None), q + 2)

    def start_writes(src_strip, src_step, dst_strip, dst_step, a):
        for ls in lanes:
            pltpu.make_async_copy(
                y_ref.at[src_strip, src_step, a, :, ls],
                o_hbm.at[dst_strip, dst_step, a, :, ls],
                sem.at[1],
            ).start()

    def write_steps(lo, hi):
        def body(t, carry):
            for a in range(2):
                start_writes(slice(None), t, slice(None), t + 1, a)
            return carry

        lax.fori_loop(lo, hi, body, 0)

    w_copy = pltpu.make_async_copy(w_hbm, w_ref, sem.at[0])
    w_copy.start()
    for r in range(4):
        for copy in row_reads(r):
            copy.start()
    for q in range(2, STEPS):
        for copy in step_reads(q):
            copy.start()
    w_copy.wait()
    _transform_filter(w_ref, u_ref)

    lane = lax.broadcasted_iota(jnp.int32, (8, 128), 1)
    even = (lane & 1) == 0
    even_wide = (jnp.concatenate([lane, lane], axis=0) & 1) == 0
    below = {n: lane < n for n in (1, 31, 32, 63, 64, 95, 96, 125, 126, 127)}
    band = {s: ((lane + s) & 96) == 96 for s in (1, 2, 3)}

    def cut(n, a, b):
        return jnp.where(below[n], a, b)

    def roll(v, s):
        return pltpu.roll(v, s, 1)

    def widen(v):
        return pltpu.bitcast(v, bf16).astype(f32)

    def row_transform(strip, q, a, e, c):
        rows = pl.ds(16 * c, 16)

        def head(s):
            return pltpu.bitcast(x0[strip[s], q, a, rows, :], u32)

        def tail(s):
            rest = pltpu.bitcast(x1[strip[s], q, a, rows, :], u32)
            return jnp.concatenate([rest, head(s)[:, 96:]], axis=1)

        def board(load, j):
            first, second = load(2 * j), load(2 * j + 1)
            return jnp.where(even, second, first), jnp.where(even, first, second)

        def emit(tile, *d):
            d = [widen(v) for v in d]
            e[tile, 0, rows] = d[0] - d[2]
            e[tile, 1, rows] = d[1] + d[2]
            e[tile, 2, rows] = d[2] - d[1]
            e[tile, 3, rows] = d[1] - d[3]

        def head_tile(j, wrap):
            other, own = board(head, j)
            emit(
                j,
                roll(cut(125, other, wrap[0]), 3),
                roll(cut(126, own, wrap[1]), 2),
                roll(cut(127, other, wrap[0]), 1),
                own,
            )

        tail_board = functools.lru_cache(None)(lambda j: board(tail, j))

        def job(j):
            filler, rest = tail_board(3), tail_board(j)
            wrap = [roll(v, 32) for v in rest]
            piece = [roll(v, 96 - 32 * j) for v in filler]

            def finish():
                def shifted(n, s):
                    return roll(jnp.where(band[s], piece[n], rest[n]), s)

                head_tile(j, wrap)
                emit(
                    4 + j,
                    shifted(0, 3),
                    shifted(1, 2),
                    shifted(0, 1),
                    cut(96, rest[1], piece[1]),
                )
                if j == 2:
                    head_tile(3, piece)

            return finish

        return [functools.partial(job, j) for j in range(3)]

    def product(e, tile, k, l, acc=None):
        def v(kl, c):
            p, q = (
                e[n // 2, n % 2, tile, kl[1], pl.ds(16 * c, 16)]
                for n in ((0, 2), (1, 2), (2, 1), (1, 3))[kl[0]]
            )
            return p + q if kl[0] == 1 else p - q

        rhs = jnp.concatenate(
            [v((k, l), c) for c in range(CHUNKS)]
            + [v(src, c) for src, c, _ in _FOLDED[k, l]],
            axis=0,
        ).astype(bf16)

        def dot(lo, size):
            lhs = u_ref[_PRODUCTS.index((k, l)), pl.ds(lo // 2, size // 2)]
            m = jnp.dot(pltpu.bitcast(lhs, bf16), rhs, preferred_element_type=f32)
            return m if acc is None else acc[lo : lo + size] + m

        if (k, l) in _HALVED:
            return jnp.concatenate([dot(0, C // 2), dot(C // 2, C // 2)], axis=0)
        return dot(0, C)

    held = {}

    def put(tile, a, b, y):
        if b == 1 and tile < 4:
            held[tile, a, b] = y
        elif tile in (1, 2):
            held[tile, a, b] = pltpu.bitcast(y.astype(bf16), u32)
        else:
            z_ref[a, b, tile] = jnp.concatenate(
                [
                    jnp.concatenate([y[r : r + 16], y[r + 16 : r + 32]], axis=1)
                    for r in range(0, C, 32)
                ],
                axis=0,
            ).astype(bf16)

    def get(tile, a, b, c):
        if b == 1 and tile < 4:
            return held[tile, a, b][16 * c : 16 * c + 16]
        if tile in (1, 2):
            return held[tile, a, b][8 * c : 8 * c + 8]
        z = z_ref[a, b, tile, pl.ds(16 * (c // 2), 16), pl.ds(128 * (c % 2), 128)]
        return pltpu.bitcast(z, u32)

    def convolve(e, tile):
        m = functools.partial(product, e, tile)
        m10, m20 = m(1, 0), m(2, 0)
        top0, bottom0 = m(0, 0, m10 + m20), m(3, 0, m10 - m20)
        m21, m12 = m(2, 1), m(1, 2)
        top1, top2 = m(0, 1, m21), m(0, 2, m12)
        minus_bottom1, bottom2 = m(3, 1, m21), m(3, 2, m12)
        top, minus_bottom = top1 - top2, minus_bottom1 + bottom2
        put(tile, 0, 0, top0 + (top + (top2 + top2)))
        put(tile, 1, 0, bottom0 + (minus_bottom - (minus_bottom1 + minus_bottom1)))

        def finish():
            m13, m23 = m(1, 3), m(2, 3)
            put(tile, 0, 1, m(0, 3, top - (m13 + m23)))
            put(tile, 1, 1, m(3, 3, (m23 - m13) - minus_bottom))

        return finish

    def convolve_tiles(e, tiles):
        for tile in tiles[:-2]:
            convolve(e, tile)()
        finish = convolve(e, tiles[-2])
        convolve(e, tiles[-1])()
        finish()

    def unpack(out, j, a, c):
        left0 = get(j, a, 0, c)
        if j < 3:
            moved = roll(get(4 + j, a, 0, c), 127)
            right1 = get(4 + j, a, 1, c)
            next0 = cut(127, roll(left0, 127), moved)
            next1 = cut(95, moved, roll(left0, 95))
        else:
            r = [roll(get(4 + i, a, 1, c), 32 * (i + 1)) for i in range(3)]
            left = [get(4, a, 0, c), get(5, a, 0, c), cut(1, left0, get(6, a, 0, c))]
            n = [roll(v, 32 * (i + 1) - 1) for i, v in enumerate(left)]
            right1 = cut(64, cut(32, r[0], r[1]), r[2])
            next0 = cut(127, roll(left0, 127), n[0])
            next1 = cut(63, cut(31, n[0], n[1]), n[2])
        head, tail = (get(j, a, 1, c), widen(next0)), (right1, next1)
        for i in range(2):
            row = jnp.concatenate(
                [
                    jnp.where(even_wide, head[i], head[1 - i]),
                    widen(jnp.where(even, tail[i], tail[1 - i])),
                ],
                axis=1,
            )
            out[2 * j + i, a, pl.ds(16 * c, 16), :] = row[:, :W].astype(bf16)

    def interleave(jobs, depth, outputs=()):
        pending, outputs = [], list(outputs)
        for n, job in enumerate(jobs):
            pending.append(job())
            while outputs and outputs[0][0] <= n:
                outputs.pop(0)[1]()
            while len(pending) > depth[n * len(depth) // len(jobs)]:
                pending.pop(0)()
        for finish in pending:
            finish()
        for _, output in outputs:
            output()

    row_chunks = [(a, c) for a in range(2) for c in range(CHUNKS)]

    def step(t, depth, spans, midway=None):
        e = e_ref.at[pl.ds(t, 3)]
        for tile in (0, 4):
            convolve(e, tile)()
        if midway:
            midway()
        convolve_tiles(e, (5, 6, 3, 1, 2))
        wrapped = (t + 2 >= STEPS).astype(jnp.int32)
        q = t + 2 - STEPS * wrapped
        strip = [(s + wrapped) & (STRIPS - 1) for s in range(STRIPS)]
        out = y_ref.at[:, t]
        interleave(
            [
                job
                for a, c in row_chunks
                for job in row_transform(strip, q, a, e.at[2, a], c)
            ],
            depth,
            [
                (lo + (hi - lo) * n / 12, functools.partial(unpack, out, j, a, c))
                for j, lo, hi in spans
                for n, (a, c) in enumerate(row_chunks)
            ],
        )

    def first_rows(r, carry):
        q, a = r >> 1, r & 1
        for copy in row_reads(r):
            copy.wait()
        interleave(
            [
                job
                for c in range(CHUNKS)
                for job in row_transform(range(STRIPS), q, a, e_ref.at[q, a], c)
            ],
            (4,),
        )
        return carry

    lax.fori_loop(0, 4, first_rows, 0)

    def phase(writing, carry):
        t0 = writing * FIRST_WRITE_STEP

        def midway():
            for copy in step_reads(t0 + 2):
                copy.wait()
            write_steps(0, t0)

        step(t0, (3,), ((0, 0, 12), (3, 24, 32), (1, 32, 36), (2, 36, 36)), midway)

        def body(t, carry):
            write_steps(t - 1, writing * t)

            @pl.when(t + 2 < STEPS)
            def _():
                for copy in step_reads(t + 2):
                    copy.wait()

            spans = ((0, 13, 27), (3, 33, 36), (1, 36, 36), (2, 36, 36))
            step(t, (2, 2, 1, 1, 2), spans)
            return carry

        end = jnp.where(writing == 0, FIRST_WRITE_STEP, STEPS - 1)
        lax.fori_loop(t0 + 1, end, body, 0)
        return carry

    lax.fori_loop(0, 2, phase, 0)

    last = STEPS - 1
    for a in range(2):
        start_writes(slice(None), last - 1, slice(None), last, a)
    for tiles, pairs in (((0, 4, 5, 6, 3), (0, 3)), ((1, 2), (1, 2))):
        convolve_tiles(e_ref.at[pl.ds(last, 2)], tiles)
        for j in pairs:
            for a, c in row_chunks:
                unpack(y_ref.at[:, last], j, a, c)
        for a in range(2):
            for s in [2 * j + i for j in pairs for i in range(2)]:
                start_writes(s, last, (s + 1) % STRIPS, 0, a)
    pltpu.make_async_copy(o_hbm, o_hbm, sem.at[1]).wait()


@jax.jit
def pallas_standalone__fft_conv__vision_kernel(
    x: jax.Array,
    w: jax.Array,
):
    assert x.shape == (1, H, W, C) and w.shape == (3, 3, C, C)
    shape = (STRIPS, STEPS, 2, C, W)
    y = pl.pallas_call(
        _kernel,
        in_specs=[pl.BlockSpec(memory_space=pl.ANY)] * 2,
        out_specs=pl.BlockSpec(memory_space=pl.ANY),
        out_shape=jax.ShapeDtypeStruct(shape, bf16),
        scratch_shapes=[
            pltpu.VMEM(shape[:-1] + (128,), bf16),
            pltpu.VMEM(shape[:-1] + (W - 128,), bf16),
            pltpu.VMEM(shape, bf16),
            pltpu.VMEM((len(_PRODUCTS), C // 2, 128), u32),
            pltpu.VMEM((STEPS + 1, 2, 7, 4, C, 128), f32),
            pltpu.VMEM((2, 2, 7, C // 2, 256), bf16),
            pltpu.VMEM((3, 3, C, C), bf16),
            pltpu.SemaphoreType.DMA((2,)),
            pltpu.SemaphoreType.DMA((STEPS + 2,)),
        ],
        compiler_params=pltpu.CompilerParams(
            vmem_limit_bytes=96 * 1024 * 1024,
            disable_semaphore_checks=True,
        ),
    )(jnp.transpose(x[0], (0, 2, 1)).reshape(shape), w)
    return jnp.transpose(y.reshape(H, C, W), (0, 2, 1))[None]
```
